```python
import os as _os
_os.environ.setdefault("JAX_PLATFORMS", "cpu")
import jax
import jax.numpy as jnp

def _softmax(x, axis=-1):
    return jax.nn.softmax(x, axis=axis)
def _gelu(x):
    return jax.nn.gelu(x, approximate=True)
def _silu(x):
    return jax.nn.silu(x)
def _sigmoid(x):
    return jax.nn.sigmoid(x)
def _layernorm(x, axis=-1, eps=1e-5):
    m = jnp.mean(x, axis=axis, keepdims=True)
    v = jnp.var(x, axis=axis, keepdims=True)
    return (x - m) / jnp.sqrt(v + eps)
def _scatter_add(tgt, idx, src, axis=0):
    return tgt.at[idx].add(src)
def _segment_sum(src, seg, n):
    return jax.ops.segment_sum(src, seg, n)
class _Rng:
    def __init__(self, key):
        self._k = key
    def _next(self):
        self._k, sub = jax.random.split(self._k)
        return sub
    def normal(self, shape):
        return jax.random.normal(self._next(), shape, dtype=jnp.bfloat16)
    def randint(self, lo, hi, shape):
        return jax.random.randint(self._next(), shape, lo, hi, dtype=jnp.int32)
    def uniform(self, shape, lo=0.0, hi=1.0):
        return jax.random.uniform(self._next(), shape, jnp.bfloat16, lo, hi)
    def permutation(self, n):
        return jax.random.permutation(self._next(), n)


kernel_name = 'gated_mix__grouped_kv_mqa__glu_gated_reglu__prompt'

def setup_inputs():
    _rng = _Rng(jax.random.key(int.from_bytes(__import__("os").urandom(4), "little")))
    _w = (lambda a: (lambda t: t.astype(jnp.bfloat16) if jnp.issubdtype(t.dtype, jnp.floating) else t)(jnp.asarray(a)))
    def _A_setup():
        B, S, D, H = 1, 2048, 640, 32
        Dh = D // H
        return {
            "x": _w((lambda *s: _rng.normal(s) * 0.05)(B, S, D)),
            "wq": _w((lambda *s: _rng.normal(s) * 0.2)(D, H * Dh)),
            "wk": _w((lambda *s: _rng.normal(s) * 0.2)(D, Dh)),
            "wv": _w((lambda *s: _rng.normal(s) * 0.05)(D, Dh)),
            "wo": _w((lambda *s: _rng.normal(s) * 0.05)(H * Dh, D)),
        }
    _A_in = _A_setup()

    def _B_setup():
        B, S, D, F = 1, 2048, 640, 1536
        return {
            "x": _w((lambda *s: _rng.normal(s) * 0.05)(B, S, D)),
            "W_gate": _w((lambda *s: _rng.normal(s) * 0.4)(D, F) * (2.0 / D) ** 0.5),
            "W_up": _w((lambda *s: _rng.normal(s) * 0.4)(D, F) * (2.0 / D) ** 0.5),
            "W_down": _w((lambda *s: _rng.normal(s) * 0.4)(F, D) * (1.0 / F) ** 0.5),
        }
    _B_in = _B_setup()

    return {
        "A_x": _A_in["x"],
        "A_wq": _A_in["wq"],
        "A_wk": _A_in["wk"],
        "A_wv": _A_in["wv"],
        "A_wo": _A_in["wo"],
        "B_x": _B_in["x"],
        "B_W_gate": _B_in["W_gate"],
        "B_W_up": _B_in["W_up"],
        "B_W_down": _B_in["W_down"],
        "gate_w": _w((lambda *s: _rng.normal(s) * 0.05)(640) * 16.0),
    }

def reference(A_x, A_wq, A_wk, A_wv, A_wo, B_x, B_W_gate, B_W_up, B_W_down, gate_w):
    def _A_ref(x, wq, wk, wv, wo):
        B, S, D = x.shape
        H = 32
        Dh = D // H
        q = (lambda x, *d: x.transpose(*d))((x @ wq).reshape(B, S, H, Dh), 0, 2, 1, 3)
        k = x @ wk
        v = x @ wv
        scores = jnp.einsum("bhqd,bkd->bhqk", q, k) * (Dh ** -0.5)
        p = _softmax(scores, axis=-1)
        o = jnp.einsum("bhqk,bkd->bhqd", p, v)
        return (lambda x, *d: x.transpose(*d))(o, 0, 2, 1, 3).reshape(B, S, H * Dh) @ wo

    def _B_ref(x, W_gate, W_up, W_down):
        gate = jnp.einsum("bsd,df->bsf", x, W_gate)
        up = jnp.einsum("bsd,df->bsf", x, W_up)
        gate = gate * (lambda x, dt: x.astype(dt))(gate > 0, gate.dtype)
        h = gate * up
        return jnp.einsum("bsf,fd->bsd", h, W_down)

    x = A_x
    g = _sigmoid((x * gate_w).sum(-1, keepdims=True))
    a = _A_ref(x, A_wq, A_wk, A_wv, A_wo)
    b = _B_ref(x, B_W_gate, B_W_up, B_W_down)
    return g * a + (1 - g) * b
```

```python
import functools
import jax
import jax.numpy as jnp
from jax.experimental import pallas as pl
from jax.experimental.pallas import tpu as pltpu

S = 2048
D = 640
H = 32
DH = 20
F = 1536
VR = 24
KD = 32
LOG2E = 1.4426950408889634
QSCALE = (DH ** -0.5) * LOG2E

bf16 = jnp.bfloat16
f32 = jnp.float32
u32 = jnp.uint32


def _dot(a, b):
    return jax.lax.dot_general(a, b, (((1,), (0,)), ((), ())), preferred_element_type=f32)


def _dot_nt(a, b):
    return jax.lax.dot_general(a, b, (((1,), (1,)), ((), ())), preferred_element_type=f32)


def _dot_tn(a, b):
    return jax.lax.dot_general(a, b, (((0,), (0,)), ((), ())), preferred_element_type=f32)


def kernel(x_hbm, wq_hbm, wkT_hbm, wvT_hbm, wo_hbm, wg_hbm, wu_hbm, wd_hbm, gw_hbm, o_ref,
           x_ref, wq_ref, wkT_ref, wvT_ref, wo_ref, wg_ref, wu_ref, wd_ref, gw_ref, sems,
           k_scr, vT_scr, qb_scr, s0_scr, s1_scr, m0_scr, m1_scr, mc_scr, oT_scr, z_ref,
           *, TQ, CK, FC, HU, XC, L, MASK):
    i = pl.program_id(0)
    NT = S // TQ
    NXC = S // XC
    NCH = S // CK

    def xcopy(c):
        return pltpu.make_async_copy(x_hbm.at[pl.ds(c * XC, XC), :], x_ref.at[pl.ds(c * XC, XC), :], sems.at[8 + c])

    small = [(wkT_hbm, wkT_ref), (wvT_hbm, wvT_ref), (wq_hbm, wq_ref), (gw_hbm, gw_ref)]
    big = [(wo_hbm, wo_ref), (wg_hbm, wg_ref), (wu_hbm, wu_ref), (wd_hbm, wd_ref)]

    def cp(k):
        src, dst = (small + big)[k]
        return pltpu.make_async_copy(src, dst, sems.at[k])

    sbuf = (s0_scr, s1_scr)
    mbuf = (m0_scr, m1_scr)

    def make_mask():
        return jax.lax.broadcasted_iota(jnp.int32, (CK, TQ), 0) >= z_ref[0]

    def a_chunk(qh, par, c, mx, mask):
        kc = pltpu.bitcast(k_scr[c * CK // 2:(c + 1) * CK // 2, :], bf16)[:, 0:KD]
        s = _dot(kc, qh)
        if MASK:
            pltpu.store(sbuf[par].at[c * CK:(c + 1) * CK, :], s, mask=mask)
        else:
            sbuf[par][c * CK:(c + 1) * CK, :] = s
        cm = jnp.max(s.reshape(CK // 8, 8, TQ), axis=0)
        mx = cm if mx is None else jnp.maximum(mx, cm)
        if c == NCH - 1:
            mbuf[par][...] = jnp.broadcast_to(jnp.max(mx, axis=0, keepdims=True), (8, TQ))
            mx = None
        return mx

    def b_chunk(par, c, m, acc):
        s = sbuf[par][c * CK:(c + 1) * CK, :].reshape(CK // 8, 8, TQ)
        p = jnp.exp2(s - m[None]).reshape(CK, TQ).astype(bf16)
        t = _dot(vT_scr[:, c * CK:(c + 1) * CK], p)
        return t if acc is None else acc + t

    @pl.when(i == 0)
    def _prologue():
        cp(0).start(); cp(1).start()
        xcopy(0).start()
        cp(2).start()
        for c in range(1, NXC):
            xcopy(c).start()
        cp(3).start()
        z_ref[0] = 0
        if MASK:
            s0_scr[...] = jnp.zeros(s0_scr.shape, f32)
            s1_scr[...] = jnp.zeros(s1_scr.shape, f32)
        cp(2).wait()
        wqT = wq_ref[...].astype(f32).T.astype(bf16)
        cp(0).wait(); cp(1).wait()
        wk_pad = jnp.concatenate([wkT_ref[...].astype(f32), jnp.zeros((128 - DH, D), f32)], axis=0).astype(bf16)
        zq = jnp.zeros((KD - DH, TQ), f32)
        for c in range(NXC):
            xcopy(c).wait()
            if c == NXC - 1:
                for k in range(4, 8):
                    cp(k).start()
            x = x_ref[c * XC:(c + 1) * XC, :]
            kk = _dot_nt(x, wk_pad).astype(bf16)
            k_scr[c * XC // 2:(c + 1) * XC // 2, :] = pltpu.bitcast(kk, u32)
            vT = _dot_nt(wvT_ref[...], x).astype(bf16).astype(f32)
            vT_scr[:, c * XC:(c + 1) * XC] = jnp.concatenate(
                [vT, jnp.ones((1, XC), f32), jnp.zeros((VR - DH - 1, XC), f32)], axis=0)
            for tt in range(XC // TQ):
                t = c * (XC // TQ) + tt
                qT = _dot_nt(wqT, x[tt * TQ:(tt + 1) * TQ]) * QSCALE
                for h in range(H):
                    qb_scr[t, h] = jnp.concatenate([qT[h * DH:(h + 1) * DH], zq], axis=0).astype(bf16)
        cp(3).wait()
        mx = None
        q0 = qb_scr[0, 0]
        for c in range(NCH):
            mx = a_chunk(q0, 0, c, mx, None if not MASK else jnp.full((CK, TQ), True))
        q1 = qb_scr[0, 1]
        mx = None
        for c in range(L):
            mx = a_chunk(q1, 1, c, mx, None if not MASK else jnp.full((CK, TQ), True))
        if L:
            mc_scr[...] = mx

    def body(j, carry):
        h0 = HU * j
        mask = make_mask() if MASK else None
        qs = []
        for u in range(1, HU + 2 if L else HU + 1):
            hn = h0 + u
            if u < HU:
                qs.append(qb_scr[i, hn])
            else:
                wrap = hn // H
                qs.append(qb_scr[jnp.minimum(i + wrap, NT - 1), hn - wrap * H])
        mx = mc_scr[...] if L else None
        outs = []
        for u in range(HU):
            m = mbuf[u % 2][...]
            acc = None
            for c in range(NCH):
                ca = c + L
                if ca < NCH:
                    mx = a_chunk(qs[u], (u + 1) % 2, ca, mx, mask)
                else:
                    mx = a_chunk(qs[u + 1], u % 2, ca - NCH, mx, mask)
                acc = b_chunk(u % 2, c, m, acc)
            outs.append(acc[0:DH] * (1.0 / acc[DH:DH + 1]))
        if L:
            mc_scr[...] = mx
        for u in range(0, HU, 2):
            r0 = pl.multiple_of(h0 * DH + u * DH, 8)
            oT_scr[pl.ds(r0, 2 * DH), :] = jnp.concatenate([outs[u], outs[u + 1]], axis=0)
        return carry

    jax.lax.fori_loop(0, H // HU, body, 0)

    @pl.when(i == 0)
    def _wait_big():
        for k in range(4, 8):
            cp(k).wait()

    row0 = pl.multiple_of(i * TQ, TQ)
    xt = x_ref[pl.ds(row0, TQ), :]
    a = _dot_tn(oT_scr[...].astype(bf16), wo_ref[...])

    b = None
    for c in range(F // FC):
        gate = _dot(xt, wg_ref[:, c * FC:(c + 1) * FC])
        up = _dot(xt, wu_ref[:, c * FC:(c + 1) * FC])
        hh = (jnp.maximum(gate, 0.0) * up).astype(bf16)
        t = _dot(hh, wd_ref[c * FC:(c + 1) * FC, :])
        b = t if b is None else b + t

    gw = gw_ref[...].reshape(1, D).astype(f32)
    g = jax.nn.sigmoid(jnp.sum(xt.astype(f32) * gw, axis=-1, keepdims=True))
    o_ref[...] = (g * a + (1.0 - g) * b).astype(o_ref.dtype)


@jax.jit
def pallas_gated_mix__grouped_kv_mqa__glu_gated_reglu__prompt_kernel(
    A_x, A_wq, A_wk, A_wv, A_wo, B_x, B_W_gate, B_W_up, B_W_down, gate_w):
    TQ, CK, FC, HU, XC, L, MASK = 256, 256, 512, 8, 512, 2, False
    x = A_x.reshape(S, D)
    hbm = pl.BlockSpec(memory_space=pl.ANY)
    out = pl.pallas_call(
        functools.partial(kernel, TQ=TQ, CK=CK, FC=FC, HU=HU, XC=XC, L=L, MASK=MASK),
        grid=(S // TQ,),
        in_specs=[hbm] * 9,
        out_specs=pl.BlockSpec((TQ, D), lambda i: (i, 0)),
        out_shape=jax.ShapeDtypeStruct((S, D), bf16),
        scratch_shapes=[
            pltpu.VMEM((S, D), bf16),
            pltpu.VMEM((D, D), bf16),
            pltpu.VMEM((DH, D), bf16),
            pltpu.VMEM((DH, D), bf16),
            pltpu.VMEM((D, D), bf16),
            pltpu.VMEM((D, F), bf16),
            pltpu.VMEM((D, F), bf16),
            pltpu.VMEM((F, D), bf16),
            pltpu.VMEM((D,), bf16),
            pltpu.SemaphoreType.DMA((8 + S // XC,)),
            pltpu.VMEM((S // 2, 128), u32),
            pltpu.VMEM((VR, S), f32),
            pltpu.VMEM((S // TQ, H, KD, TQ), bf16),
            pltpu.VMEM((S, TQ), f32),
            pltpu.VMEM((S, TQ), f32),
            pltpu.VMEM((8, TQ), f32),
            pltpu.VMEM((8, TQ), f32),
            pltpu.VMEM((8, TQ), f32),
            pltpu.VMEM((D, TQ), f32),
            pltpu.SMEM((1,), jnp.int32),
        ],
        compiler_params=pltpu.CompilerParams(
            dimension_semantics=("arbitrary",),
            vmem_limit_bytes=100 * 1024 * 1024),
    )(x, A_wq, A_wk.T, A_wv.T, A_wo, B_W_gate, B_W_up, B_W_down, gate_w)
    return out.reshape(1, S, D)
```

```python
import functools

import jax
import jax.numpy as jnp
from jax.experimental import pallas as pl
from jax.experimental.pallas import tpu as pltpu

S = 2048
D = 640
H = 32
DH = 20
F = 1536
VR = 24
KD = 32
TQ = 256
NT = S // TQ
CK = 128
NCH = S // CK
LAG = 4
FC = 512
XCS = (512, 1536)
LOG2E = 1.4426950408889634
QSCALE = (DH ** -0.5) * LOG2E

bf16 = jnp.bfloat16
f32 = jnp.float32
u32 = jnp.uint32


def _dot(a, b):
    return jax.lax.dot_general(a, b, (((1,), (0,)), ((), ())), preferred_element_type=f32)


def _dot_nt(a, b):
    return jax.lax.dot_general(a, b, (((1,), (1,)), ((), ())), preferred_element_type=f32)


def _dot_tn(a, b):
    return jax.lax.dot_general(a, b, (((0,), (0,)), ((), ())), preferred_element_type=f32)


def _kernel(x_hbm, wq_hbm, wkT_hbm, wvT_hbm, wo_hbm, wg_hbm, wu_hbm, wd_hbm, gw_hbm, o_ref,
            x_ref, wq_ref, wkT_ref, wvT_ref, wo_ref, wg_ref, wu_ref, wd_ref, gw_ref, sems,
            k_scr, vT_scr, qb_scr, s0_scr, s1_scr, m0_scr, m1_scr, mc_scr, oT_scr):
    i = pl.program_id(0)
    xoff = [sum(XCS[:c]) for c in range(len(XCS) + 1)]
    weights = [(wq_hbm, wq_ref), (wkT_hbm, wkT_ref), (wvT_hbm, wvT_ref), (gw_hbm, gw_ref),
               (wo_hbm, wo_ref), (wg_hbm, wg_ref), (wu_hbm, wu_ref), (wd_hbm, wd_ref)]

    def wcopy(k):
        src, dst = weights[k]
        return pltpu.make_async_copy(src, dst, sems.at[k])

    def xcopy(c):
        rows = pl.ds(xoff[c], XCS[c])
        return pltpu.make_async_copy(x_hbm.at[rows, :], x_ref.at[rows, :], sems.at[len(weights) + c])

    sbuf = (s0_scr, s1_scr)
    mbuf = (m0_scr, m1_scr)

    def a_chunk(qh, par, c, mx):
        kc = pltpu.bitcast(k_scr[c * CK // 2:(c + 1) * CK // 2, :], bf16)[:, 0:KD]
        s = _dot(kc, qh)
        sbuf[par][c * CK:(c + 1) * CK, :] = s
        cm = jnp.max(s.reshape(CK // 8, 8, TQ), axis=0)
        mx = cm if mx is None else jnp.maximum(mx, cm)
        if c == NCH - 1:
            mbuf[par][...] = jnp.broadcast_to(jnp.max(mx, axis=0, keepdims=True), (8, TQ))
            mx = None
        return mx

    def b_chunk(par, c, m, acc):
        s = sbuf[par][c * CK:(c + 1) * CK, :].reshape(CK // 8, 8, TQ)
        p = jnp.exp2(s - m[None]).reshape(CK, TQ).astype(bf16)
        t = _dot(vT_scr[:, c * CK:(c + 1) * CK], p)
        return t if acc is None else acc + t

    @pl.when(i == 0)
    def _prologue():
        for k in range(3):
            wcopy(k).start()
        for c in range(len(XCS)):
            xcopy(c).start()
        for k in range(3, len(weights)):
            wcopy(k).start()
        for k in range(3):
            wcopy(k).wait()
        xcopy(0).wait()
        zpad = jnp.zeros((4, D), f32)
        wall = jnp.concatenate(
            [wq_ref[...].astype(f32).T, wkT_ref[...].astype(f32), zpad,
             wvT_ref[...].astype(f32), zpad], axis=0).astype(bf16)
        zq = jnp.zeros((KD - DH, TQ), f32)
        for c in range(len(XCS)):
            if c > 0:
                xcopy(c).wait()
            for t in range(xoff[c] // TQ, xoff[c + 1] // TQ):
                pr = _dot_nt(wall, x_ref[t * TQ:(t + 1) * TQ, :])
                qT = pr[0:D] * QSCALE
                for h in range(H):
                    qb_scr[t, h] = jnp.concatenate(
                        [qT[h * DH:(h + 1) * DH], zq], axis=0).astype(bf16)
                kT = jnp.concatenate([pr[D:D + 24], jnp.zeros((128 - 24, TQ), f32)], axis=0)
                k_scr[t * TQ // 2:(t + 1) * TQ // 2, :] = pltpu.bitcast(kT.T.astype(bf16), u32)
                vT = pr[D + 24:D + 24 + DH].astype(bf16).astype(f32)
                vT_scr[:, t * TQ:(t + 1) * TQ] = jnp.concatenate(
                    [vT, jnp.ones((1, TQ), f32), jnp.zeros((VR - DH - 1, TQ), f32)], axis=0)
        mx = None
        q0 = qb_scr[0, 0]
        for c in range(NCH):
            mx = a_chunk(q0, 0, c, mx)
        q1 = qb_scr[0, 1]
        for c in range(LAG):
            mx = a_chunk(q1, 1, c, mx)
        mc_scr[...] = mx
        for k in range(3, len(weights)):
            wcopy(k).wait()

    nxt = jnp.minimum(i + 1, NT - 1)
    qs = [qb_scr[i, h] for h in range(1, H)] + [qb_scr[nxt, 0], qb_scr[nxt, 1]]
    mx = mc_scr[...]
    outs = []
    for h in range(H):
        m = mbuf[h % 2][...]
        acc = None
        for c in range(NCH):
            ca = c + LAG
            if ca < NCH:
                mx = a_chunk(qs[h], (h + 1) % 2, ca, mx)
            else:
                mx = a_chunk(qs[h + 1], h % 2, ca - NCH, mx)
            acc = b_chunk(h % 2, c, m, acc)
        outs.append(acc[0:DH] * (1.0 / acc[DH:DH + 1]))
    mc_scr[...] = mx
    for h in range(0, H, 2):
        oT_scr[h * DH:(h + 2) * DH, :] = jnp.concatenate([outs[h], outs[h + 1]], axis=0)

    xt = x_ref[pl.ds(pl.multiple_of(i * TQ, TQ), TQ), :]
    a = _dot_tn(oT_scr[...].astype(bf16), wo_ref[...])

    b = None
    for c in range(F // FC):
        gate = _dot(xt, wg_ref[:, c * FC:(c + 1) * FC])
        up = _dot(xt, wu_ref[:, c * FC:(c + 1) * FC])
        hh = (jnp.maximum(gate, 0.0) * up).astype(bf16)
        t = _dot(hh, wd_ref[c * FC:(c + 1) * FC, :])
        b = t if b is None else b + t

    gw = gw_ref[...].reshape(1, D).astype(f32)
    g = jax.nn.sigmoid(jnp.sum(xt.astype(f32) * gw, axis=-1, keepdims=True))
    o_ref[...] = (g * a + (1.0 - g) * b).astype(o_ref.dtype)


@jax.jit
def pallas_gated_mix__grouped_kv_mqa__glu_gated_reglu__prompt_kernel(
    A_x: jax.Array,
    A_wq: jax.Array,
    A_wk: jax.Array,
    A_wv: jax.Array,
    A_wo: jax.Array,
    B_x: jax.Array,
    B_W_gate: jax.Array,
    B_W_up: jax.Array,
    B_W_down: jax.Array,
    gate_w: jax.Array,
):
    del B_x
    hbm = pl.BlockSpec(memory_space=pl.ANY)
    out = pl.pallas_call(
        _kernel,
        grid=(NT,),
        in_specs=[hbm] * 9,
        out_specs=pl.BlockSpec((TQ, D), lambda i: (i, 0)),
        out_shape=jax.ShapeDtypeStruct((S, D), bf16),
        scratch_shapes=[
            pltpu.VMEM((S, D), bf16),
            pltpu.VMEM((D, D), bf16),
            pltpu.VMEM((DH, D), bf16),
            pltpu.VMEM((DH, D), bf16),
            pltpu.VMEM((D, D), bf16),
            pltpu.VMEM((D, F), bf16),
            pltpu.VMEM((D, F), bf16),
            pltpu.VMEM((F, D), bf16),
            pltpu.VMEM((D,), bf16),
            pltpu.SemaphoreType.DMA((8 + len(XCS),)),
            pltpu.VMEM((S // 2, 128), u32),
            pltpu.VMEM((VR, S), f32),
            pltpu.VMEM((NT, H, KD, TQ), bf16),
            pltpu.VMEM((S, TQ), f32),
            pltpu.VMEM((S, TQ), f32),
            pltpu.VMEM((8, TQ), f32),
            pltpu.VMEM((8, TQ), f32),
            pltpu.VMEM((8, TQ), f32),
            pltpu.VMEM((D, TQ), f32),
        ],
        compiler_params=pltpu.CompilerParams(
            dimension_semantics=("arbitrary",),
            vmem_limit_bytes=100 * 1024 * 1024),
    )(A_x.reshape(S, D), A_wq, A_wk.T, A_wv.T, A_wo, B_W_gate, B_W_up, B_W_down, gate_w)
    return out.reshape(1, S, D)
```

```python
import jax
import jax.numpy as jnp
from jax.experimental import pallas as pl
from jax.experimental.pallas import tpu as pltpu

S = 2048
D = 640
H = 32
DH = 20
F = 1536
VR = 24
KD = 32
TQ = 256
NT = S // TQ
CK = 128
NCH = S // CK
LAG = 6
CV = 16
NV = CV * (NCH // 2)
FC = 256
TP = 512
WR = D + 48
LOG2E = 1.4426950408889634
QSCALE = (DH ** -0.5) * LOG2E

bf16 = jnp.bfloat16
f32 = jnp.float32
u32 = jnp.uint32


def _dot(a, b):
    return jax.lax.dot_general(a, b, (((1,), (0,)), ((), ())), preferred_element_type=f32)


def _dot_nt(a, b):
    return jax.lax.dot_general(a, b, (((1,), (1,)), ((), ())), preferred_element_type=f32)


def _dot_tn(a, b):
    return jax.lax.dot_general(a, b, (((0,), (0,)), ((), ())), preferred_element_type=f32)


def _kernel(x_hbm, wq_hbm, wkT_hbm, wvT_hbm, wo_hbm, wg_hbm, wu_hbm, wd_hbm, gw_hbm, o_ref,
            x_ref, wq_ref, wkT_ref, wvT_ref, wo_ref, wg_ref, wu_ref, wd_ref, gw_ref, sems,
            wall_scr, k_scr, vT_scr, qb_scr, kb_scr, qv_scr,
            s0_scr, s1_scr, m0_scr, m1_scr, mc_scr, oT_scr):
    i = pl.program_id(0)
    weights = [(wq_hbm, wq_ref), (wkT_hbm, wkT_ref), (wvT_hbm, wvT_ref), (gw_hbm, gw_ref),
               (wo_hbm, wo_ref), (wg_hbm, wg_ref), (wu_hbm, wu_ref), (wd_hbm, wd_ref)]
    xrows = [pl.ds(0, TP), pl.ds(TP, S - TP)]

    def wcopy(k):
        src, dst = weights[k]
        return pltpu.make_async_copy(src, dst, sems.at[k])

    def xcopy(c):
        return pltpu.make_async_copy(x_hbm.at[xrows[c], :], x_ref.at[xrows[c], :],
                                     sems.at[len(weights) + c])

    sbuf = (s0_scr, s1_scr)
    mbuf = (m0_scr, m1_scr)

    def a_chunk(q, par, c, mx):
        qh, slot = q
        cv = CV if c % 2 == 0 else 0
        cm = CK - cv
        if cv:
            r0 = (c // 2) * CV
            halves = [None] * (TQ // 128)
            for d in range(DH):
                kb = kb_scr[d, r0:r0 + cv, :]
                for n, l0 in enumerate(range(0, TQ, 128)):
                    t = kb * qv_scr[slot, d:d + 1, l0:l0 + 128]
                    halves[n] = t if halves[n] is None else halves[n] + t
            sv = jnp.concatenate(halves, axis=1)
            sbuf[par][c * CK + cm:(c + 1) * CK, :] = sv
            vm = jnp.max(sv.reshape(cv // 8, 8, TQ), axis=0)
            mx = vm if mx is None else jnp.maximum(mx, vm)
        kc = pltpu.bitcast(k_scr[c * CK // 2:(c * CK + cm) // 2, :], bf16)[:, 0:KD]
        s = _dot(kc, qh)
        sbuf[par][c * CK:c * CK + cm, :] = s
        sm = jnp.max(s.reshape(cm // 8, 8, TQ), axis=0)
        mx = sm if mx is None else jnp.maximum(mx, sm)
        if c == NCH - 1:
            mbuf[par][...] = jnp.broadcast_to(jnp.max(mx, axis=0, keepdims=True), (8, TQ))
            mx = None
        return mx

    def b_chunk(par, c, m, acc):
        s = sbuf[par][c * CK:(c + 1) * CK, :].reshape(CK // 8, 8, TQ)
        p = jnp.exp2(s - m[None]).reshape(CK, TQ).astype(bf16)
        t = _dot(vT_scr[:, c * CK:(c + 1) * CK], p)
        return t if acc is None else acc + t

    @pl.when(i == 0)
    def _prologue():
        for k in range(3):
            wcopy(k).start()
        xcopy(0).start()
        xcopy(1).start()
        for k in range(3, len(weights)):
            wcopy(k).start()
        for k in range(3):
            wcopy(k).wait()
        xcopy(0).wait()
        zpad = jnp.zeros((4, D), f32)
        wall = jnp.concatenate(
            [wq_ref[...].astype(f32).T, wkT_ref[...].astype(f32), zpad,
             wvT_ref[...].astype(f32), zpad], axis=0).astype(bf16)
        wall_scr[...] = wall
        zq = jnp.zeros((KD - DH, TQ), f32)

        def proj(tp, w):
            hint = (lambda v, m: v) if isinstance(tp, int) else pl.multiple_of
            r0 = hint(tp * TP, TP)
            pr = _dot_nt(w, x_ref[pl.ds(r0, TP), :])
            qT = pr[0:D] * QSCALE
            for tt in range(TP // TQ):
                for h in range(H):
                    qb_scr[tp * (TP // TQ) + tt, h] = jnp.concatenate(
                        [qT[h * DH:(h + 1) * DH, tt * TQ:(tt + 1) * TQ], zq], axis=0).astype(bf16)
            kT = jnp.concatenate([pr[D:D + 24], jnp.zeros((128 - 24, TP), f32)], axis=0)
            k_scr[pl.ds(hint(tp * (TP // 2), TP // 2), TP // 2), :] = pltpu.bitcast(
                kT.T.astype(bf16), u32)
            vT = pr[D + 24:D + 24 + DH].astype(bf16).astype(f32)
            vT_scr[:, pl.ds(r0, TP)] = jnp.concatenate(
                [vT, jnp.ones((1, TP), f32), jnp.zeros((VR - DH - 1, TP), f32)], axis=0)

        proj(0, wall)
        xcopy(1).wait()

        def proj_loop(tp, carry):
            proj(tp, wall_scr[...])
            return carry

        jax.lax.fori_loop(1, S // TP, proj_loop, 0)

        kall = pltpu.bitcast(k_scr[...], bf16)
        sel = jax.lax.broadcasted_iota(jnp.int32, (128, 128), 0)
        for c in range(0, NCH, 2):
            kv = kall[(c + 1) * CK - CV:(c + 1) * CK, :]
            for d in range(DH):
                kb_scr[d, (c // 2) * CV:(c // 2 + 1) * CV, :] = _dot(kv, (sel == d).astype(bf16))

        q0 = qb_scr[0, 0]
        q1 = qb_scr[0, 1]
        qv_scr[0] = q0.astype(f32)
        qv_scr[1] = q1.astype(f32)
        mx = None
        for c in range(NCH):
            mx = a_chunk((q0, 0), 0, c, mx)
        for c in range(LAG):
            mx = a_chunk((q1, 1), 1, c, mx)
        mc_scr[...] = mx
        for k in range(3, len(weights)):
            wcopy(k).wait()

    xt = x_ref[pl.ds(pl.multiple_of(i * TQ, TQ), TQ), :]

    def ffn_piece(c, b):
        gate = _dot(xt, wg_ref[:, c * FC:(c + 1) * FC])
        up = _dot(xt, wu_ref[:, c * FC:(c + 1) * FC])
        hh = (jnp.maximum(gate, 0.0) * up).astype(bf16)
        t = _dot(hh, wd_ref[c * FC:(c + 1) * FC, :])
        return t if b is None else b + t

    npieces = F // FC
    piece_after = {((2 * c + 1) * H) // (2 * npieces): c for c in range(npieces)}

    nxt = jnp.minimum(i + 1, NT - 1)
    qs = [qb_scr[i, h] for h in range(1, H)] + [qb_scr[nxt, 0], qb_scr[nxt, 1]]
    for k in range(len(qs)):
        qv_scr[k] = qs[k].astype(f32)
    qs = [(q, k) for k, q in enumerate(qs)]
    mx = mc_scr[...]
    outs = []
    b = None
    for h in range(H):
        m = mbuf[h % 2][...]
        acc = None
        for c in range(NCH):
            ca = c + LAG
            if ca < NCH:
                mx = a_chunk(qs[h], (h + 1) % 2, ca, mx)
            else:
                mx = a_chunk(qs[h + 1], h % 2, ca - NCH, mx)
            acc = b_chunk(h % 2, c, m, acc)
        outs.append(acc[0:DH] * (1.0 / acc[DH:DH + 1]))
        if h in piece_after:
            b = ffn_piece(piece_after[h], b)
    mc_scr[...] = mx
    for h in range(0, H, 2):
        oT_scr[h * DH:(h + 2) * DH, :] = jnp.concatenate([outs[h], outs[h + 1]], axis=0)

    a = _dot_tn(oT_scr[...].astype(bf16), wo_ref[...])
    gw = gw_ref[...].reshape(1, D).astype(f32)
    g = jax.nn.sigmoid(jnp.sum(xt.astype(f32) * gw, axis=-1, keepdims=True))
    o_ref[...] = (g * a + (1.0 - g) * b).astype(o_ref.dtype)


@jax.jit
def pallas_gated_mix__grouped_kv_mqa__glu_gated_reglu__prompt_kernel(
    A_x: jax.Array,
    A_wq: jax.Array,
    A_wk: jax.Array,
    A_wv: jax.Array,
    A_wo: jax.Array,
    B_x: jax.Array,
    B_W_gate: jax.Array,
    B_W_up: jax.Array,
    B_W_down: jax.Array,
    gate_w: jax.Array,
):
    del B_x
    hbm = pl.BlockSpec(memory_space=pl.ANY)
    out = pl.pallas_call(
        _kernel,
        grid=(NT,),
        in_specs=[hbm] * 9,
        out_specs=pl.BlockSpec((TQ, D), lambda i: (i, 0)),
        out_shape=jax.ShapeDtypeStruct((S, D), bf16),
        scratch_shapes=[
            pltpu.VMEM((S, D), bf16),
            pltpu.VMEM((D, D), bf16),
            pltpu.VMEM((DH, D), bf16),
            pltpu.VMEM((DH, D), bf16),
            pltpu.VMEM((D, D), bf16),
            pltpu.VMEM((D, F), bf16),
            pltpu.VMEM((D, F), bf16),
            pltpu.VMEM((F, D), bf16),
            pltpu.VMEM((D,), bf16),
            pltpu.SemaphoreType.DMA((10,)),
            pltpu.VMEM((WR, D), bf16),
            pltpu.VMEM((S // 2, 128), u32),
            pltpu.VMEM((VR, S), f32),
            pltpu.VMEM((NT, H, KD, TQ), bf16),
            pltpu.VMEM((DH, NV, 128), f32),
            pltpu.VMEM((H + 1, KD, TQ), f32),
            pltpu.VMEM((S, TQ), f32),
            pltpu.VMEM((S, TQ), f32),
            pltpu.VMEM((8, TQ), f32),
            pltpu.VMEM((8, TQ), f32),
            pltpu.VMEM((8, TQ), f32),
            pltpu.VMEM((D, TQ), f32),
        ],
        compiler_params=pltpu.CompilerParams(
            dimension_semantics=("arbitrary",),
            vmem_limit_bytes=100 * 1024 * 1024),
    )(A_x.reshape(S, D), A_wq, A_wk.T, A_wv.T, A_wo, B_W_gate, B_W_up, B_W_down, gate_w)
    return out.reshape(1, S, D)
```
